```python
import os as _os
_os.environ.setdefault("JAX_PLATFORMS", "cpu")
import jax
import jax.numpy as jnp

def _softmax(x, axis=-1):
    return jax.nn.softmax(x, axis=axis)
def _gelu(x):
    return jax.nn.gelu(x, approximate=True)
def _silu(x):
    return jax.nn.silu(x)
def _sigmoid(x):
    return jax.nn.sigmoid(x)
def _layernorm(x, axis=-1, eps=1e-5):
    m = jnp.mean(x, axis=axis, keepdims=True)
    v = jnp.var(x, axis=axis, keepdims=True)
    return (x - m) / jnp.sqrt(v + eps)
def _scatter_add(tgt, idx, src, axis=0):
    return tgt.at[idx].add(src)
def _segment_sum(src, seg, n):
    return jax.ops.segment_sum(src, seg, n)
class _Rng:
    def __init__(self, key):
        self._k = key
    def _next(self):
        self._k, sub = jax.random.split(self._k)
        return sub
    def normal(self, shape):
        return jax.random.normal(self._next(), shape, dtype=jnp.bfloat16)
    def randint(self, lo, hi, shape):
        return jax.random.randint(self._next(), shape, lo, hi, dtype=jnp.int32)
    def uniform(self, shape, lo=0.0, hi=1.0):
        return jax.random.uniform(self._next(), shape, jnp.bfloat16, lo, hi)
    def permutation(self, n):
        return jax.random.permutation(self._next(), n)


kernel_name = 'standalone__mha_softmax__near_ridge'

def setup_inputs():
    _rng = _Rng(jax.random.key(int.from_bytes(__import__("os").urandom(4), "little")))
    _w = (lambda a: (lambda t: t.astype(jnp.bfloat16) if jnp.issubdtype(t.dtype, jnp.floating) else t)(jnp.asarray(a)))
    B, H, Sq, Sk, D = 16, 16, 256, 256, 256
    return {
        "q": _w((lambda *s: _rng.normal(s) * 0.4)(B, H, Sq, D)),
        "k": _w((lambda *s: _rng.normal(s) * 0.4)(B, H, Sk, D)),
        "v": _w((lambda *s: _rng.normal(s) * 0.05)(B, H, Sk, D)),
    }

def reference(q, k, v):
    scale = q.shape[-1] ** -0.5
    scores = jnp.einsum("bhqd,bhkd->bhqk", q, k) * scale
    p = _softmax(scores, axis=-1)
    return jnp.einsum("bhqk,bhkd->bhqd", p, v)
```

```python
import jax
import jax.numpy as jnp
import jax.experimental.pallas as pl
import jax.experimental.pallas.tpu as pltpu


def _mha_kernel(q_ref, k_ref, v_ref, o_ref, *, scale, heads_per_step):
    for h in range(heads_per_step):
        q = q_ref[h]
        k = k_ref[h]
        v = v_ref[h]
        s = jax.lax.dot_general(
            q, k, (((1,), (1,)), ((), ())), preferred_element_type=jnp.float32
        ) * scale
        m = jnp.max(s, axis=-1, keepdims=True)
        p = jnp.exp(s - m)
        l = jnp.sum(p, axis=-1, keepdims=True)
        o = jnp.dot(p.astype(v.dtype), v, preferred_element_type=jnp.float32)
        o_ref[h] = (o / l).astype(o_ref.dtype)


@jax.jit
def pallas_standalone__mha_softmax__near_ridge_kernel(
    q: jax.Array,
    k: jax.Array,
    v: jax.Array,
):
    B, H, Sq, D = q.shape
    Sk = k.shape[2]
    Dv = v.shape[3]
    BH = B * H
    scale = float(D) ** -0.5
    hb = 4
    while BH % hb:
        hb //= 2

    q3 = q.reshape(BH, Sq, D)
    k3 = k.reshape(BH, Sk, D)
    v3 = v.reshape(BH, Sk, Dv)

    def kernel(q_ref, k_ref, v_ref, o_ref):
        _mha_kernel(q_ref, k_ref, v_ref, o_ref, scale=scale, heads_per_step=hb)

    out = pl.pallas_call(
        kernel,
        grid=(BH // hb,),
        in_specs=[
            pl.BlockSpec((hb, Sq, D), lambda i: (i, 0, 0)),
            pl.BlockSpec((hb, Sk, D), lambda i: (i, 0, 0)),
            pl.BlockSpec((hb, Sk, Dv), lambda i: (i, 0, 0)),
        ],
        out_specs=pl.BlockSpec((hb, Sq, Dv), lambda i: (i, 0, 0)),
        out_shape=jax.ShapeDtypeStruct((BH, Sq, Dv), q.dtype),
        compiler_params=pltpu.CompilerParams(
            dimension_semantics=("parallel",),
        ),
    )(q3, k3, v3)
    return out.reshape(B, H, Sq, Dv)
```

```python
import jax
import jax.numpy as jnp
from jax import lax
from jax.experimental import pallas as pl
from jax.experimental.pallas import tpu as pltpu

_VMEM_LIMIT_BYTES = 110 * 1024 * 1024
_VMEM_BUDGET_BYTES = 96 * 1024 * 1024
_MAX_REGIONS = 8
_MAX_HEADS_PER_REGION_STEP = 2
_WRITE_ROWS = 64
_WRITES_IN_FLIGHT = 8
_WRITES_PER_TAIL_HEAD = 2


def _attend(q, k, v, scale):
    s = lax.dot_general(
        q, k, (((1,), (1,)), ((), ())), preferred_element_type=jnp.float32
    ) * scale
    m = jnp.max(s, axis=-1, keepdims=True)
    p = jnp.exp(s - m)
    l = jnp.sum(p, axis=-1, keepdims=True)
    o = jnp.dot(p.astype(v.dtype), v, preferred_element_type=jnp.float32)
    return o / l


def _largest_divisor(n, cap):
    return max(d for d in range(1, min(n, cap) + 1) if n % d == 0)


def _staged_plan(bh, sq, sk, d, dv, itemsize):
    ns = _largest_divisor(bh, _MAX_REGIONS)
    hps = bh // ns
    hpr = _largest_divisor(hps, _MAX_HEADS_PER_REGION_STEP)
    if hps // hpr < 2 and hpr > 1:
        hpr = 1
    n = hps // hpr
    if n < 2:
        return None
    sublanes = 8 * max(1, 4 // itemsize)
    wrows = _WRITE_ROWS
    while wrows > sublanes and sq % wrows:
        wrows //= 2
    if sq % wrows or sq % sublanes or dv % 128:
        return None
    hb = ns * hpr
    staged = bh * sq * dv * itemsize
    inputs = 2 * hb * (sq * d + sk * d + sk * dv) * itemsize
    temps = 6 * sq * max(sk, dv) * 4
    if staged + inputs + temps > _VMEM_BUDGET_BYTES:
        return None
    return ns, hps, hpr, n, wrows


def _staged_call_args(sq, sk, d, dv, dtype, scale, plan):
    ns, hps, hpr, n, wrows = plan
    nf = _WRITES_IN_FLIGHT
    tail_rows = hpr * sq
    main_rows = (n - 1) * tail_rows
    nw = (main_rows + tail_rows) // wrows
    nw_main = main_rows // wrows

    def kernel(q_ref, k_ref, v_ref, o_hbm, o_main, o_tail, sems):
        i = pl.program_id(0)

        def write_dma(t):
            if t < nw_main:
                src = o_main.at[:, pl.ds(t * wrows, wrows), :]
            else:
                src = o_tail.at[:, pl.ds((t - nw_main) * wrows, wrows), :]
            dst = o_hbm.at[:, pl.ds(t * wrows, wrows), :]
            return pltpu.make_async_copy(src, dst, sems.at[t % nf])

        def start_next(started, limit):
            if started >= limit:
                return started
            if started >= nf:
                write_dma(started - nf).wait()
            write_dma(started).start()
            return started + 1

        def head(r, j):
            o = _attend(q_ref[r, j], k_ref[r, j], v_ref[r, j], scale)
            return o.astype(dtype)

        @pl.when(i < n - 1)
        def _():
            step = jnp.minimum(i, n - 2)
            for r in range(ns):
                for j in range(hpr):
                    row = pl.multiple_of((step * hpr + j) * sq, sq)
                    o_main[r, pl.ds(row, sq), :] = head(r, j)

        @pl.when(i == n - 1)
        def _():
            started = 0
            for _ in range(nf):
                started = start_next(started, nw_main)
            for r in range(ns):
                for j in range(hpr):
                    o_tail[r, pl.ds(j * sq, sq), :] = head(r, j)
                    for _ in range(_WRITES_PER_TAIL_HEAD):
                        started = start_next(started, nw_main)
            while started < nw:
                started = start_next(started, nw)
            for t in range(max(0, nw - nf), nw):
                write_dma(t).wait()

    return dict(
        kernel=kernel,
        grid=(n,),
        in_specs=[
            pl.BlockSpec((ns, hpr, sq, d), lambda i: (0, i, 0, 0)),
            pl.BlockSpec((ns, hpr, sk, d), lambda i: (0, i, 0, 0)),
            pl.BlockSpec((ns, hpr, sk, dv), lambda i: (0, i, 0, 0)),
        ],
        out_specs=pl.BlockSpec(memory_space=pl.ANY),
        out_shape=jax.ShapeDtypeStruct((ns, hps * sq, dv), dtype),
        scratch_shapes=[
            pltpu.VMEM((ns, main_rows, dv), dtype),
            pltpu.VMEM((ns, tail_rows, dv), dtype),
            pltpu.SemaphoreType.DMA((nf,)),
        ],
        semantics=("arbitrary",),
    )


def _pipelined_call_args(bh, sq, sk, d, dv, dtype, scale):
    hb = _largest_divisor(bh, 4)

    def kernel(q_ref, k_ref, v_ref, o_ref):
        for h in range(hb):
            o_ref[h] = _attend(q_ref[h], k_ref[h], v_ref[h], scale).astype(dtype)

    return dict(
        kernel=kernel,
        grid=(bh // hb,),
        in_specs=[
            pl.BlockSpec((hb, sq, d), lambda i: (i, 0, 0)),
            pl.BlockSpec((hb, sk, d), lambda i: (i, 0, 0)),
            pl.BlockSpec((hb, sk, dv), lambda i: (i, 0, 0)),
        ],
        out_specs=pl.BlockSpec((hb, sq, dv), lambda i: (i, 0, 0)),
        out_shape=jax.ShapeDtypeStruct((bh, sq, dv), dtype),
        scratch_shapes=[],
        semantics=("parallel",),
    )


@jax.jit
def pallas_standalone__mha_softmax__near_ridge_kernel(
    q: jax.Array,
    k: jax.Array,
    v: jax.Array,
):
    B, H, Sq, D = q.shape
    Sk = k.shape[2]
    Dv = v.shape[3]
    BH = B * H
    dtype = q.dtype
    scale = float(D) ** -0.5

    plan = _staged_plan(BH, Sq, Sk, D, Dv, jnp.dtype(dtype).itemsize)
    if plan is not None:
        ns, hps = plan[0], plan[1]
        args = _staged_call_args(Sq, Sk, D, Dv, dtype, scale, plan)
        lead = (ns, hps)
    else:
        args = _pipelined_call_args(BH, Sq, Sk, D, Dv, dtype, scale)
        lead = (BH,)

    out = pl.pallas_call(
        args["kernel"],
        grid=args["grid"],
        in_specs=args["in_specs"],
        out_specs=args["out_specs"],
        out_shape=args["out_shape"],
        scratch_shapes=args["scratch_shapes"],
        compiler_params=pltpu.CompilerParams(
            dimension_semantics=args["semantics"],
            vmem_limit_bytes=_VMEM_LIMIT_BYTES,
        ),
    )(
        q.reshape(lead + (Sq, D)),
        k.reshape(lead + (Sk, D)),
        v.reshape(lead + (Sk, Dv)),
    )
    return out.reshape(B, H, Sq, Dv)
```
